```python
import os as _os
_os.environ.setdefault("JAX_PLATFORMS", "cpu")
import jax
import jax.numpy as jnp

def _softmax(x, axis=-1):
    return jax.nn.softmax(x, axis=axis)
def _gelu(x):
    return jax.nn.gelu(x, approximate=True)
def _silu(x):
    return jax.nn.silu(x)
def _sigmoid(x):
    return jax.nn.sigmoid(x)
def _layernorm(x, axis=-1, eps=1e-5):
    m = jnp.mean(x, axis=axis, keepdims=True)
    v = jnp.var(x, axis=axis, keepdims=True)
    return (x - m) / jnp.sqrt(v + eps)
def _scatter_add(tgt, idx, src, axis=0):
    return tgt.at[idx].add(src)
def _segment_sum(src, seg, n):
    return jax.ops.segment_sum(src, seg, n)
class _Rng:
    def __init__(self, key):
        self._k = key
    def _next(self):
        self._k, sub = jax.random.split(self._k)
        return sub
    def normal(self, shape):
        return jax.random.normal(self._next(), shape, dtype=jnp.bfloat16)
    def randint(self, lo, hi, shape):
        return jax.random.randint(self._next(), shape, lo, hi, dtype=jnp.int32)
    def uniform(self, shape, lo=0.0, hi=1.0):
        return jax.random.uniform(self._next(), shape, jnp.bfloat16, lo, hi)
    def permutation(self, n):
        return jax.random.permutation(self._next(), n)


kernel_name = 'standalone__gqa_softmax__near_ridge'

def setup_inputs():
    _rng = _Rng(jax.random.key(int.from_bytes(__import__("os").urandom(4), "little")))
    _w = (lambda a: (lambda t: t.astype(jnp.bfloat16) if jnp.issubdtype(t.dtype, jnp.floating) else t)(jnp.asarray(a)))
    B, Hq, Hkv, Sq, Sk, D = 8, 16, 8, 512, 512, 256
    return {
        "q": _w((lambda *s: _rng.normal(s) * 0.4)(B, Hq, Sq, D)),
        "k": _w((lambda *s: _rng.normal(s) * 0.4)(B, Hkv, Sk, D)),
        "v": _w((lambda *s: _rng.normal(s) * 0.05)(B, Hkv, Sk, D)),
    }

def reference(q, k, v):
    B, Hq, Sq, D = q.shape
    Hkv = k.shape[1]
    rep = Hq // Hkv
    k = jnp.repeat(k, rep, axis=1)
    v = jnp.repeat(v, rep, axis=1)
    scale = D ** -0.5
    scores = jnp.einsum("bhqd,bhkd->bhqk", q, k) * scale
    p = _softmax(scores, axis=-1)
    return jnp.einsum("bhqk,bhkd->bhqd", p, v)
```

```python
import math

import jax
import jax.numpy as jnp
from jax import lax
import jax.experimental.pallas as pl
import jax.experimental.pallas.tpu as pltpu

_GROUP = 16
_IN_SLOTS = 4
_OUT_SLOTS = 2
_BQ = 128
_LOOKAHEAD = 2
_Q0_CHUNKS = (256, 256, 512)
_O_LAST_CHUNK = 128


@jax.jit
def pallas_standalone__gqa_softmax__near_ridge_kernel(
    q: jax.Array,
    k: jax.Array,
    v: jax.Array,
):
    B, Hq, Sq, D = q.shape
    Hkv, Sk = k.shape[1], k.shape[2]
    N = B * Hkv
    M = (Hq // Hkv) * Sq
    G, R, RO, bq, la = _GROUP, _IN_SLOTS, _OUT_SLOTS, _BQ, _LOOKAHEAD
    U = M // bq
    NG = N // G
    assert N % G == 0 and G % R == 0 and G % RO == 0 and M % bq == 0
    assert sum(_Q0_CHUNKS) == M
    q0_starts = [sum(_Q0_CHUNKS[:i]) for i in range(len(_Q0_CHUNKS))]
    c = (D**-0.5) * math.log2(math.e)

    def kernel(q_hbm, k_hbm, v_hbm, o_hbm, q_buf, k_buf, v_buf, o_buf,
               qsem, q0sem, ksem, vsem, osem):

        def q_starts(j):
            return q0_starts if j % G == 0 else [0]

        def q_copy(h, j, r0):
            s = j % R
            if j % G == 0:
                i = q0_starts.index(r0)
                rows = pl.ds(r0, _Q0_CHUNKS[i])
                return pltpu.make_async_copy(
                    q_hbm.at[h, rows], q_buf.at[s, rows], q0sem.at[i])
            return pltpu.make_async_copy(q_hbm.at[h], q_buf.at[s], qsem.at[s])

        def k_copy(h, j):
            return pltpu.make_async_copy(
                k_hbm.at[h], k_buf.at[j % R], ksem.at[j % R])

        def v_copy(h, j):
            return pltpu.make_async_copy(
                v_hbm.at[h], v_buf.at[j % R], vsem.at[j % R])

        def o_wait(j):
            pltpu.make_async_copy(
                o_buf.at[j % RO], o_hbm.at[0], osem.at[j % RO]).wait()

        def maybe(always, cond, fn):
            if always:
                fn()
            else:
                pl.when(cond)(fn)

        for j in range(R):
            k_copy(j, j).start()
            for r0 in q_starts(j):
                if r0 < (la + 1) * bq:
                    q_copy(j, j, r0).start()
            v_copy(j, j).start()
            for r0 in q_starts(j):
                if r0 >= (la + 1) * bq:
                    q_copy(j, j, r0).start()

        def body(g, carry):
            n = G * U
            probs = {}
            for t in range(n + la):
                if t < n:
                    j, i = divmod(t, U)
                    h = g * G + j
                    if i == 0:
                        k_copy(h, j).wait()
                    if i * bq in q_starts(j):
                        q_copy(h, j, i * bq).wait()
                    s = lax.dot_general(
                        q_buf[j % R, i * bq:(i + 1) * bq, :], k_buf[j % R],
                        (((1,), (1,)), ((), ())),
                        preferred_element_type=jnp.float32)
                    if i == U - 1:

                        def prefetch_kq(h=h, j=j):
                            k_copy(h + R, j + R).start()
                            for r0 in q_starts(j + R):
                                q_copy(h + R, j + R, r0).start()

                        maybe(j + R < G, g + 1 < NG, prefetch_kq)
                    m = jnp.max(s, axis=-1, keepdims=True)
                    p = jnp.exp2((s - m) * c)
                    l = jnp.sum(p, axis=-1, keepdims=True)
                    probs[t] = (p * (1.0 / l)).astype(v_buf.dtype)
                if t >= la:
                    j, i = divmod(t - la, U)
                    h = g * G + j
                    if i == 0:
                        v_copy(h, j).wait()
                        maybe(j >= RO, g > 0, lambda j=j: o_wait(j))
                    o = jnp.dot(probs.pop(t - la), v_buf[j % R],
                                preferred_element_type=jnp.float32)
                    if i == U - 1:
                        maybe(j + R < G, g + 1 < NG,
                              lambda h=h, j=j: v_copy(h + R, j + R).start())
                    o_buf[j % RO, i * bq:(i + 1) * bq, :] = o.astype(o_buf.dtype)
                    oc = _O_LAST_CHUNK if j == G - 1 else M
                    r1 = (i + 1) * bq
                    if r1 % oc == 0:
                        rows = pl.ds(r1 - oc, oc)
                        pltpu.make_async_copy(
                            o_buf.at[j % RO, rows], o_hbm.at[h, rows],
                            osem.at[j % RO]).start()
            return carry

        lax.fori_loop(0, NG, body, 0)
        for j in range(RO):
            o_wait(j)

    out = pl.pallas_call(
        kernel,
        in_specs=[pl.BlockSpec(memory_space=pl.ANY)] * 3,
        out_specs=pl.BlockSpec(memory_space=pl.ANY),
        out_shape=jax.ShapeDtypeStruct((N, M, D), q.dtype),
        scratch_shapes=[
            pltpu.VMEM((R, M, D), q.dtype),
            pltpu.VMEM((R, Sk, D), k.dtype),
            pltpu.VMEM((R, Sk, D), v.dtype),
            pltpu.VMEM((RO, M, D), q.dtype),
            pltpu.SemaphoreType.DMA((R,)),
            pltpu.SemaphoreType.DMA((len(_Q0_CHUNKS),)),
            pltpu.SemaphoreType.DMA((R,)),
            pltpu.SemaphoreType.DMA((R,)),
            pltpu.SemaphoreType.DMA((RO,)),
        ],
        compiler_params=pltpu.CompilerParams(
            vmem_limit_bytes=100 * 2**20,
            flags={"XLA_TPU_RESCHEDULE_DMA_DONES": True},
            disable_bounds_checks=True,
        ),
    )(q.reshape(N, M, D), k.reshape(N, Sk, D), v.reshape(N, Sk, D))
    return out.reshape(B, Hq, Sq, D)
```

```python
import math

import jax
import jax.numpy as jnp
from jax import lax
import jax.experimental.pallas as pl
import jax.experimental.pallas.tpu as pltpu

_GROUP = 16
_SLOTS = 4
_BQ = 128
_AHEAD = 2
_AHEAD_FIRST = 3
_FIRST_Q_UNITS = (1, 1, 2)
_LAST_ROWS = 32


@jax.jit
def pallas_standalone__gqa_softmax__near_ridge_kernel(
    q: jax.Array,
    k: jax.Array,
    v: jax.Array,
):
    B, Hq, Sq, D = q.shape
    Hkv, Sk = k.shape[1], k.shape[2]
    N = B * Hkv
    M = (Hq // Hkv) * Sq
    G, R, bq = _GROUP, _SLOTS, _BQ
    U = M // bq
    NG = N // G
    T = G * U
    assert N % G == 0 and G % R == 0 and M % bq == 0
    assert sum(_FIRST_Q_UNITS) == _AHEAD_FIRST + 1 < U
    c = (D**-0.5) * math.log2(math.e)

    order = [("qk", t) for t in range(_AHEAD_FIRST + 1)]
    order += [("pv", t) for t in range(_AHEAD_FIRST - _AHEAD + 1)]
    for t in range(_AHEAD_FIRST + 1, T):
        order += [("qk", t), ("pv", t - _AHEAD)]
    order += [("pv", t) for t in range(T - _AHEAD, T)]

    k_row, v_row = M, M + Sk
    whole = [("k", 0, k_row, Sk), ("q", 0, 0, M), ("v", 0, v_row, Sk)]
    pieces = [("k", 0, k_row, Sk)]
    row = 0
    for units in _FIRST_Q_UNITS:
        pieces.append(("q", row, row, units * bq))
        row += units * bq
    pieces += [("v", 0, v_row, Sk), ("q", row, row, M - row)]

    def kernel(q_hbm, k_hbm, v_hbm, o_hbm, in_buf, o_buf,
               piece_sems, in_sems, o_sems):
        hbm = {"q": q_hbm, "k": k_hbm, "v": v_hbm}

        def in_copy(h, j, part, sem):
            name, src_row, dst_row, rows = part
            return pltpu.make_async_copy(
                hbm[name].at[h, pl.ds(src_row, rows)],
                in_buf.at[j % R, pl.ds(dst_row, rows)], sem)

        def start_inputs(h, j):
            if j % G == 0:
                for n, part in enumerate(pieces):
                    in_copy(h, j, part, piece_sems.at[n]).start()
            else:
                for part in whole:
                    in_copy(h, j, part, in_sems.at[j % R]).start()

        def wait_piece(h, name, src_row):
            for n, part in enumerate(pieces):
                if part[:2] == (name, src_row):
                    in_copy(h, 0, part, piece_sems.at[n]).wait()

        def wait_slot(buf, sems, j):
            slot = buf.at[j % R]
            pltpu.make_async_copy(slot, slot, sems.at[j % R]).wait()

        def run_if(always, cond, fn):
            if always:
                fn()
            else:
                pl.when(cond)(fn)

        def qk_softmax(h, j, i):
            if j == 0:
                if i == 0:
                    wait_piece(h, "k", 0)
                wait_piece(h, "q", i * bq)
            elif i == 0:
                wait_slot(in_buf, in_sems, j)
            s = lax.dot_general(
                in_buf[j % R, pl.ds(i * bq, bq)],
                in_buf[j % R, pl.ds(k_row, Sk)],
                (((1,), (1,)), ((), ())),
                preferred_element_type=jnp.float32)
            m = jnp.max(s, axis=-1, keepdims=True)
            p = jnp.exp2((s - m) * c)
            l = jnp.sum(p, axis=-1, keepdims=True)
            return (p * pltpu.reciprocal(l, full_range=False)).astype(v_hbm.dtype)

        def pv_store(g, h, j, i, p):
            if i == 0:
                if j == 0:
                    wait_piece(h, "v", 0)
                run_if(j >= R, g > 0, lambda: wait_slot(o_buf, o_sems, j))
            o = jnp.dot(p, in_buf[j % R, pl.ds(v_row, Sk)],
                        preferred_element_type=jnp.float32).astype(o_buf.dtype)
            if i == U - 1:
                run_if(j + R < G, g + 1 < NG,
                       lambda: start_inputs(h + R, j + R))
            if j < G - 1:
                copy_rows = M
            else:
                copy_rows = bq if i < U - 1 else _LAST_ROWS
            step = min(copy_rows, bq)
            for a in range(0, bq, step):
                end = i * bq + a + step
                o_buf[j % R, pl.ds(end - step, step)] = o[a:a + step]
                if end % copy_rows == 0:
                    rows = pl.ds(end - copy_rows, copy_rows)
                    pltpu.make_async_copy(
                        o_buf.at[j % R, rows], o_hbm.at[h, rows],
                        o_sems.at[j % R]).start()

        def group(g, carry):
            probs = {}
            for kind, t in order:
                j, i = divmod(t, U)
                h = g * G + j
                if kind == "qk":
                    probs[t] = qk_softmax(h, j, i)
                else:
                    pv_store(g, h, j, i, probs.pop(t))
            return carry

        for j in range(R):
            start_inputs(j, j)
        lax.fori_loop(0, NG, group, 0)
        for j in range(R):
            wait_slot(o_buf, o_sems, j)

    out = pl.pallas_call(
        kernel,
        in_specs=[pl.BlockSpec(memory_space=pl.ANY)] * 3,
        out_specs=pl.BlockSpec(memory_space=pl.ANY),
        out_shape=jax.ShapeDtypeStruct((N, M, D), q.dtype),
        scratch_shapes=[
            pltpu.VMEM((R, M + 2 * Sk, D), q.dtype),
            pltpu.VMEM((R, M, D), q.dtype),
            pltpu.SemaphoreType.DMA((len(pieces),)),
            pltpu.SemaphoreType.DMA((R,)),
            pltpu.SemaphoreType.DMA((R,)),
        ],
        compiler_params=pltpu.CompilerParams(
            vmem_limit_bytes=100 * 2**20,
            flags={"XLA_TPU_RESCHEDULE_DMA_DONES": True},
            disable_bounds_checks=True,
            disable_semaphore_checks=True,
        ),
    )(q.reshape(N, M, D), k.reshape(N, Sk, D), v.reshape(N, Sk, D))
    return out.reshape(B, Hq, Sq, D)
```
